```python
import os as _os
_os.environ.setdefault("JAX_PLATFORMS", "cpu")
import jax
import jax.numpy as jnp

def _softmax(x, axis=-1):
    return jax.nn.softmax(x, axis=axis)
def _gelu(x):
    return jax.nn.gelu(x, approximate=True)
def _silu(x):
    return jax.nn.silu(x)
def _sigmoid(x):
    return jax.nn.sigmoid(x)
def _layernorm(x, axis=-1, eps=1e-5):
    m = jnp.mean(x, axis=axis, keepdims=True)
    v = jnp.var(x, axis=axis, keepdims=True)
    return (x - m) / jnp.sqrt(v + eps)
def _scatter_add(tgt, idx, src, axis=0):
    return tgt.at[idx].add(src)
def _segment_sum(src, seg, n):
    return jax.ops.segment_sum(src, seg, n)
class _Rng:
    def __init__(self, key):
        self._k = key
    def _next(self):
        self._k, sub = jax.random.split(self._k)
        return sub
    def normal(self, shape):
        return jax.random.normal(self._next(), shape, dtype=jnp.bfloat16)
    def randint(self, lo, hi, shape):
        return jax.random.randint(self._next(), shape, lo, hi, dtype=jnp.int32)
    def uniform(self, shape, lo=0.0, hi=1.0):
        return jax.random.uniform(self._next(), shape, jnp.bfloat16, lo, hi)
    def permutation(self, n):
        return jax.random.permutation(self._next(), n)


kernel_name = 'standalone__instancenorm__sampling'

def setup_inputs():
    _rng = _Rng(jax.random.key(int.from_bytes(__import__("os").urandom(4), "little")))
    _w = (lambda a: (lambda t: t.astype(jnp.bfloat16) if jnp.issubdtype(t.dtype, jnp.floating) else t)(jnp.asarray(a)))
    B, C, H, W = 16, 640, 16, 32
    return {
        "x": _w((lambda *s: _rng.normal(s) * 0.05)(B, C, H, W)),
        "g": _w((lambda *s: _rng.normal(s) * 0.05)(C) + 1.0),
        "b": _w((lambda *s: _rng.normal(s) * 0.05)(C)),
    }

def reference(x, g, b):
    mu = x.mean(axis=(-2, -1), keepdims=True)
    var = ((x - mu) * (x - mu)).mean(axis=(-2, -1), keepdims=True)
    xhat = (x - mu) / jnp.sqrt(var + 1e-5)
    return xhat * g.reshape(1, -1, 1, 1) + b.reshape(1, -1, 1, 1)
```

```python
import jax
import jax.numpy as jnp
import jax.experimental.pallas as pl
import jax.experimental.pallas.tpu as pltpu

EPS = 1e-5


def _kernel(x_ref, g_ref, b_ref, o_ref):
    x = x_ref[0].astype(jnp.float32)
    n = x.shape[0]
    mu = jnp.sum(x, axis=0, keepdims=True) * (1.0 / n)
    xc = x - mu
    var = jnp.sum(xc * xc, axis=0, keepdims=True) * (1.0 / n)
    scale = g_ref[...].astype(jnp.float32) * jax.lax.rsqrt(var + EPS)
    o_ref[0] = (xc * scale + b_ref[...].astype(jnp.float32)).astype(o_ref.dtype)


@jax.jit
def pallas_standalone__instancenorm__sampling_kernel(
    x: jax.Array,
    g: jax.Array,
    b: jax.Array,
):
    B, C, H, W = x.shape
    HW = H * W
    xt = jnp.transpose(x, (0, 2, 3, 1)).reshape(B, HW, C)
    g2 = g.reshape(1, C)
    b2 = b.reshape(1, C)
    out = pl.pallas_call(
        _kernel,
        grid=(B,),
        in_specs=[
            pl.BlockSpec((1, HW, C), lambda i: (i, 0, 0)),
            pl.BlockSpec((1, C), lambda i: (0, 0)),
            pl.BlockSpec((1, C), lambda i: (0, 0)),
        ],
        out_specs=pl.BlockSpec((1, HW, C), lambda i: (i, 0, 0)),
        out_shape=jax.ShapeDtypeStruct((B, HW, C), x.dtype),
        compiler_params=pltpu.CompilerParams(
            dimension_semantics=("parallel",),
        ),
    )(xt, g2, b2)
    return jnp.transpose(out.reshape(B, H, W, C), (0, 3, 1, 2))
```

```python
import functools

import jax
import jax.numpy as jnp
import jax.experimental.pallas as pl
import jax.experimental.pallas.tpu as pltpu

EPS = 1e-5

PIECE_ROWS = 16
ROW_CHUNK = 128
FIRST_READ = 6
READ_TAIL = 16
WRITE_SPLITS = (6, 11, 16)


def _kernel(x_hbm, g_hbm, b_hbm, o_hbm, xbuf, gbuf, bbuf, dbuf, sems):
    B, S, M, C = xbuf.shape
    HW = S * M
    spc = ROW_CHUNK // M
    nchunk = HW // ROW_CHUNK
    n0 = FIRST_READ
    last = B - 1
    head = S - READ_TAIL

    r0 = [
        pltpu.make_async_copy(g_hbm, gbuf, sems.at[0]),
        pltpu.make_async_copy(b_hbm, bbuf, sems.at[0]),
        pltpu.make_async_copy(
            x_hbm.at[pl.ds(0, n0)], xbuf.at[pl.ds(0, n0)], sems.at[0]),
    ]
    r1 = [
        pltpu.make_async_copy(
            x_hbm.at[pl.ds(n0, last - n0)], xbuf.at[pl.ds(n0, last - n0)],
            sems.at[1]),
        pltpu.make_async_copy(
            x_hbm.at[last, pl.ds(0, head)], xbuf.at[last, pl.ds(0, head)],
            sems.at[1]),
    ]
    r2 = pltpu.make_async_copy(
        x_hbm.at[last, pl.ds(head, READ_TAIL)],
        xbuf.at[last, pl.ds(head, READ_TAIL)], sems.at[2])

    def start_writes(lo, hi):
        def body(j, carry):
            idx = (pl.ds(lo, hi - lo), j)
            pltpu.make_async_copy(xbuf.at[idx], o_hbm.at[idx], sems.at[3]).start()
            return carry
        jax.lax.fori_loop(0, S, body, 0)

    def wait_r1():
        for c in r1:
            c.wait()

    bounds = (0,) + WRITE_SPLITS
    events = {i: [] for i in range(B + 1)}
    events[1].append(lambda: r2.start(priority=1))
    events[n0].append(wait_r1)
    events[n0].append(functools.partial(start_writes, bounds[0], bounds[1]))
    events[last].append(r2.wait)
    for k in range(1, len(WRITE_SPLITS)):
        events[bounds[k + 1]].append(
            functools.partial(start_writes, bounds[k], bounds[k + 1]))

    def run_events(evs):
        for ev in evs:
            ev()

    for c in r0:
        c.start(priority=0)
    for c in r1:
        c.start(priority=1)
    for c in r0:
        c.wait()

    gamma = gbuf[...].astype(jnp.float32).reshape(1, C)
    beta = bbuf[...].astype(jnp.float32).reshape(1, C)

    def norm_batch(i, carry):
        for j in range(B):
            if events[j]:
                pl.when(i == j)(functools.partial(run_events, events[j]))

        def load(j):
            s0 = pl.multiple_of(j * spc, spc)
            return xbuf[i, pl.ds(s0, spc)].astype(jnp.float32).reshape(ROW_CHUNK, C)

        def rows(j):
            return pl.ds(pl.multiple_of(j * ROW_CHUNK, ROW_CHUNK), ROW_CHUNK)

        def mean_step(j, acc):
            return acc + jnp.sum(load(j).reshape(ROW_CHUNK // 8, 8, C), axis=0)
        acc = jax.lax.fori_loop(0, nchunk, mean_step, jnp.zeros((8, C), jnp.float32))
        mu = jnp.sum(acc, axis=0, keepdims=True) * (1.0 / HW)

        def var_step(j, acc):
            d = load(j) - mu
            dbuf[rows(j), :] = d
            return acc + jnp.sum((d * d).reshape(ROW_CHUNK // 8, 8, C), axis=0)
        acc = jax.lax.fori_loop(0, nchunk, var_step, jnp.zeros((8, C), jnp.float32))
        var = jnp.sum(acc, axis=0, keepdims=True) * (1.0 / HW)
        scale = gamma * jax.lax.rsqrt(var + EPS)

        def out_step(j, c):
            s0 = pl.multiple_of(j * spc, spc)
            y = dbuf[rows(j), :] * scale + beta
            xbuf[i, pl.ds(s0, spc)] = y.astype(xbuf.dtype).reshape(spc, M, C)
            return c
        jax.lax.fori_loop(0, nchunk, out_step, 0)
        return carry

    jax.lax.fori_loop(0, B, norm_batch, 0)
    run_events(events[B])
    pltpu.make_async_copy(xbuf, o_hbm, sems.at[3]).wait()


@jax.jit
def pallas_standalone__instancenorm__sampling_kernel(
    x: jax.Array,
    g: jax.Array,
    b: jax.Array,
):
    B, C, H, W = x.shape
    HW = H * W
    S = HW // PIECE_ROWS
    xt = jnp.transpose(x, (0, 2, 3, 1)).reshape(B, S, PIECE_ROWS, C)
    out = pl.pallas_call(
        _kernel,
        in_specs=[pl.BlockSpec(memory_space=pl.ANY)] * 3,
        out_specs=pl.BlockSpec(memory_space=pl.ANY),
        out_shape=jax.ShapeDtypeStruct(xt.shape, x.dtype),
        scratch_shapes=[
            pltpu.VMEM(xt.shape, x.dtype),
            pltpu.VMEM((C,), g.dtype),
            pltpu.VMEM((C,), b.dtype),
            pltpu.VMEM((HW, C), jnp.float32),
            pltpu.SemaphoreType.DMA((4,)),
        ],
        compiler_params=pltpu.CompilerParams(
            vmem_limit_bytes=32 * 1024 * 1024,
        ),
    )(xt, g, b)
    return jnp.transpose(out.reshape(B, H, W, C), (0, 3, 1, 2))
```

```python
import functools

import jax
import jax.numpy as jnp
import jax.experimental.pallas as pl
import jax.experimental.pallas.tpu as pltpu

EPS = 1e-5

PIECE_ROWS = 16
ROW_CHUNK = 128
FIRST_READ = 6
READ_TAIL = 18
WRITE_SPLITS = (6, 11, 16)


def _kernel(x_hbm, g_hbm, b_hbm, o_hbm, xbuf, gbuf, bbuf, dbuf, sems):
    B, S, M, C = xbuf.shape
    HW = S * M
    spc = ROW_CHUNK // M
    nchunk = HW // ROW_CHUNK
    n0 = FIRST_READ
    last = B - 1
    head = S - READ_TAIL

    r0 = [
        pltpu.make_async_copy(g_hbm, gbuf, sems.at[0]),
        pltpu.make_async_copy(b_hbm, bbuf, sems.at[0]),
        pltpu.make_async_copy(
            x_hbm.at[pl.ds(0, n0)], xbuf.at[pl.ds(0, n0)], sems.at[0]),
    ]
    r1 = [
        pltpu.make_async_copy(
            x_hbm.at[pl.ds(n0, last - n0)], xbuf.at[pl.ds(n0, last - n0)],
            sems.at[1]),
        pltpu.make_async_copy(
            x_hbm.at[last, pl.ds(0, head)], xbuf.at[last, pl.ds(0, head)],
            sems.at[1]),
    ]
    r2 = pltpu.make_async_copy(
        x_hbm.at[last, pl.ds(head, READ_TAIL)],
        xbuf.at[last, pl.ds(head, READ_TAIL)], sems.at[0])

    def start_writes(lo, hi):
        def body(j, carry):
            idx = (pl.ds(lo, hi - lo), j)
            pltpu.make_async_copy(xbuf.at[idx], o_hbm.at[idx], sems.at[1]).start()
            return carry
        jax.lax.fori_loop(0, S, body, 0)

    def wait_r1():
        for c in r1:
            c.wait()

    bounds = (0,) + WRITE_SPLITS
    events = {i: [] for i in range(B + 1)}
    events[1].append(lambda: r2.start(priority=1))
    events[n0].append(wait_r1)
    events[n0].append(functools.partial(start_writes, bounds[0], bounds[1]))
    events[last].append(r2.wait)
    for k in range(1, len(WRITE_SPLITS)):
        events[bounds[k + 1]].append(
            functools.partial(start_writes, bounds[k], bounds[k + 1]))

    def run_events(evs):
        for ev in evs:
            ev()

    for c in r0:
        c.start(priority=0)
    for c in r1:
        c.start(priority=1)
    for c in r0:
        c.wait()

    gamma = gbuf[...].astype(jnp.float32).reshape(1, C)
    beta = bbuf[...].astype(jnp.float32).reshape(1, C)

    def norm_batch(i, carry):
        for j in range(B):
            if events[j]:
                pl.when(i == j)(functools.partial(run_events, events[j]))

        def load(j):
            s0 = pl.multiple_of(j * spc, spc)
            return xbuf[i, pl.ds(s0, spc)].astype(jnp.float32).reshape(ROW_CHUNK, C)

        def rows(j):
            return pl.ds(pl.multiple_of(j * ROW_CHUNK, ROW_CHUNK), ROW_CHUNK)

        def mean_step(j, acc):
            return acc + jnp.sum(load(j).reshape(ROW_CHUNK // 8, 8, C), axis=0)
        acc = jax.lax.fori_loop(0, nchunk, mean_step, jnp.zeros((8, C), jnp.float32))
        mu = jnp.sum(acc, axis=0, keepdims=True) * (1.0 / HW)

        def var_step(j, acc):
            d = load(j) - mu
            dbuf[rows(j), :] = d
            return acc + jnp.sum((d * d).reshape(ROW_CHUNK // 8, 8, C), axis=0)
        acc = jax.lax.fori_loop(0, nchunk, var_step, jnp.zeros((8, C), jnp.float32))
        var = jnp.sum(acc, axis=0, keepdims=True) * (1.0 / HW)
        scale = gamma * jax.lax.rsqrt(var + EPS)

        def out_step(j, c):
            s0 = pl.multiple_of(j * spc, spc)
            y = dbuf[rows(j), :] * scale + beta
            xbuf[i, pl.ds(s0, spc)] = y.astype(xbuf.dtype).reshape(spc, M, C)
            return c
        jax.lax.fori_loop(0, nchunk, out_step, 0)
        return carry

    jax.lax.fori_loop(0, B, norm_batch, 0)
    run_events(events[B])
    pltpu.make_async_copy(xbuf, o_hbm, sems.at[1]).wait()


@jax.jit
def pallas_standalone__instancenorm__sampling_kernel(
    x: jax.Array,
    g: jax.Array,
    b: jax.Array,
):
    B, C, H, W = x.shape
    HW = H * W
    S = HW // PIECE_ROWS
    xt = jnp.transpose(x, (0, 2, 3, 1)).reshape(B, S, PIECE_ROWS, C)
    out = pl.pallas_call(
        _kernel,
        in_specs=[pl.BlockSpec(memory_space=pl.ANY)] * 3,
        out_specs=pl.BlockSpec(memory_space=pl.ANY),
        out_shape=jax.ShapeDtypeStruct(xt.shape, x.dtype),
        scratch_shapes=[
            pltpu.VMEM(xt.shape, x.dtype),
            pltpu.VMEM((C,), g.dtype),
            pltpu.VMEM((C,), b.dtype),
            pltpu.VMEM((HW, C), jnp.float32),
            pltpu.SemaphoreType.DMA((2,)),
        ],
        compiler_params=pltpu.CompilerParams(
            vmem_limit_bytes=32 * 1024 * 1024,
        ),
    )(xt, g, b)
    return jnp.transpose(out.reshape(B, H, W, C), (0, 3, 1, 2))
```
